```python
import os as _os
_os.environ.setdefault("JAX_PLATFORMS", "cpu")
import jax
import jax.numpy as jnp

def _softmax(x, axis=-1):
    return jax.nn.softmax(x, axis=axis)
def _gelu(x):
    return jax.nn.gelu(x, approximate=True)
def _silu(x):
    return jax.nn.silu(x)
def _sigmoid(x):
    return jax.nn.sigmoid(x)
def _layernorm(x, axis=-1, eps=1e-5):
    m = jnp.mean(x, axis=axis, keepdims=True)
    v = jnp.var(x, axis=axis, keepdims=True)
    return (x - m) / jnp.sqrt(v + eps)
def _scatter_add(tgt, idx, src, axis=0):
    return tgt.at[idx].add(src)
def _segment_sum(src, seg, n):
    return jax.ops.segment_sum(src, seg, n)
class _Rng:
    def __init__(self, key):
        self._k = key
    def _next(self):
        self._k, sub = jax.random.split(self._k)
        return sub
    def normal(self, shape):
        return jax.random.normal(self._next(), shape, dtype=jnp.bfloat16)
    def randint(self, lo, hi, shape):
        return jax.random.randint(self._next(), shape, lo, hi, dtype=jnp.int32)
    def uniform(self, shape, lo=0.0, hi=1.0):
        return jax.random.uniform(self._next(), shape, jnp.bfloat16, lo, hi)
    def permutation(self, n):
        return jax.random.permutation(self._next(), n)


kernel_name = 'concat_heads__mha_block_cached__mha_block_cached__near_ridge'

def setup_inputs():
    _rng = _Rng(jax.random.key(int.from_bytes(__import__("os").urandom(4), "little")))
    _w = (lambda a: (lambda t: t.astype(jnp.bfloat16) if jnp.issubdtype(t.dtype, jnp.floating) else t)(jnp.asarray(a)))
    def _A_setup():
        B, Sq, D = 16, 32, 1024
        H, Sk, Dh = 32, 32, 128
        return {
            "x": _w((lambda *s: _rng.normal(s) * 0.8)(B, Sq, D)),
            "k_cache": _w((lambda *s: _rng.normal(s) * 0.8)(B, H, Sk, Dh)),
            "v_cache": _w((lambda *s: _rng.normal(s) * 0.05)(B, H, Sk, Dh)),
            "wq": _w((lambda *s: _rng.normal(s) * 0.8)(D, H * Dh) * (D ** -0.5)),
            "wo": _w((lambda *s: _rng.normal(s) * 0.05)(H * Dh, D) * ((H * Dh) ** -0.5)),
        }
    _A_in = _A_setup()

    def _B_setup():
        B, Sq, D = 16, 32, 1024
        H, Sk, Dh = 32, 32, 128
        return {
            "x": _w((lambda *s: _rng.normal(s) * 0.8)(B, Sq, D)),
            "k_cache": _w((lambda *s: _rng.normal(s) * 0.8)(B, H, Sk, Dh)),
            "v_cache": _w((lambda *s: _rng.normal(s) * 0.05)(B, H, Sk, Dh)),
            "wq": _w((lambda *s: _rng.normal(s) * 0.8)(D, H * Dh) * (D ** -0.5)),
            "wo": _w((lambda *s: _rng.normal(s) * 0.05)(H * Dh, D) * ((H * Dh) ** -0.5)),
        }
    _B_in = _B_setup()

    return {
        "A_x": _A_in["x"],
        "A_k_cache": _A_in["k_cache"],
        "A_v_cache": _A_in["v_cache"],
        "A_wq": _A_in["wq"],
        "A_wo": _A_in["wo"],
        "B_x": _B_in["x"],
        "B_k_cache": _B_in["k_cache"],
        "B_v_cache": _B_in["v_cache"],
        "B_wq": _B_in["wq"],
        "B_wo": _B_in["wo"],
    }

def reference(A_x, A_k_cache, A_v_cache, A_wq, A_wo, B_x, B_k_cache, B_v_cache, B_wq, B_wo):
    def _A_ref(x, k_cache, v_cache, wq, wo):
        B, Sq, D = x.shape
        H, Dh = 32, 128
        q = (lambda x, *d: x.transpose(*d))((x @ wq).reshape(B, Sq, H, Dh), 0, 2, 1, 3)
        scores = jnp.einsum("bhqd,bhkd->bhqk", q, k_cache) * (Dh ** -0.5)
        p = _softmax(scores, axis=-1)
        o = jnp.einsum("bhqk,bhkd->bhqd", p, v_cache)
        return (lambda x, *d: x.transpose(*d))(o, 0, 2, 1, 3).reshape(B, Sq, H * Dh) @ wo

    def _B_ref(x, k_cache, v_cache, wq, wo):
        B, Sq, D = x.shape
        H, Dh = 32, 128
        q = (lambda x, *d: x.transpose(*d))((x @ wq).reshape(B, Sq, H, Dh), 0, 2, 1, 3)
        scores = jnp.einsum("bhqd,bhkd->bhqk", q, k_cache) * (Dh ** -0.5)
        p = _softmax(scores, axis=-1)
        o = jnp.einsum("bhqk,bhkd->bhqd", p, v_cache)
        return (lambda x, *d: x.transpose(*d))(o, 0, 2, 1, 3).reshape(B, Sq, H * Dh) @ wo

    a = _A_ref(A_x, A_k_cache, A_v_cache, A_wq, A_wo)
    b = _B_ref(B_x, B_k_cache, B_v_cache, B_wq, B_wo)
    return jnp.concatenate([a, b], axis=-1)
```

```python
import jax
import jax.numpy as jnp
from jax import lax
import jax.experimental.pallas as pl
import jax.experimental.pallas.tpu as pltpu

B, SQ, D = 16, 32, 1024
H, SK, DH = 32, 32, 128
M = B * SQ
HU = 4
UW = HU * DH
HG = 16
GW = HG * DH
NG = 4
EXP2_SCALE = (DH ** -0.5) * 1.4426950408889634
F32 = jnp.float32
BF16 = jnp.bfloat16


def _scores(q_ref, k_ref, t, p_ref):
    lane_grp = lax.broadcasted_iota(jnp.int32, (SK, 128), 1) // SQ
    for g in range(4):
        pts = []
        for h in range(HU * t, HU * (t + 1)):
            kh = k_ref[4 * g:4 * g + 4, h].reshape(128, DH)
            qh = q_ref[128 * g:128 * (g + 1), DH * h:DH * (h + 1)]
            st = lax.dot_general(kh, qh, (((1,), (1,)), ((), ())), preferred_element_type=F32)
            d = st[0:SK]
            for j in range(1, 4):
                d = jnp.where(lane_grp == j, st[SK * j:SK * (j + 1)], d)
            m = jnp.max(d, axis=0, keepdims=True)
            e = jnp.exp2((d - m) * EXP2_SCALE)
            l = jnp.sum(e, axis=0, keepdims=True)
            pts.append(e * (1.0 / l))
        pt = jnp.concatenate(pts, axis=0)
        p_ref[128 * g:128 * (g + 1), :] = pt.T.astype(BF16)


def _pv(p_ref, v_ref, t, o_ref):
    lane_grp = lax.broadcasted_iota(jnp.int32, (SQ, 128), 1) // SK
    for b in range(B):
        pb = p_ref[SQ * b:SQ * (b + 1), :]
        zero = jnp.zeros_like(pb)
        pe = jnp.concatenate([jnp.where(lane_grp == h, pb, zero) for h in range(HU)], axis=0)
        vb = v_ref[b, HU * t:HU * (t + 1)].reshape(128, DH)
        ob = jnp.dot(pe, vb, preferred_element_type=F32).astype(BF16)
        for h in range(HU):
            o_ref[SQ * b:SQ * (b + 1), DH * h:DH * (h + 1)] = ob[SQ * h:SQ * (h + 1)]


def _kernel(xa, ka, va, wqa, woa, xb, kb, vb, wqb, wob, out_hbm,
            x_buf, wq_buf, wo_buf, k_buf, v_buf, q_buf, p_buf, o_buf, acc, out_buf,
            sems):
    class _S:
        def __init__(self, base): self.base = base
        @property
        def at(self): return self
        def __getitem__(self, i): return sems.at[self.base + i]
    sem_x, sem_wq0, sem_wq, sem_wo, sem_k, sem_v, sem_out = _S(0), _S(2), _S(5), _S(9), _S(13), _S(17), _S(21)
    xs, ks, vs, wqs, wos = (xa, xb), (ka, kb), (va, vb), (wqa, wqb), (woa, wob)

    def cp_x(br):
        return pltpu.make_async_copy(xs[br], x_buf.at[br], sem_x.at[br])

    W0 = [(0, 512), (512, 512), (1024, 1024)]

    def cp_wq0(c):
        s, w = W0[c]
        return pltpu.make_async_copy(wqa.at[:, pl.ds(s, w)], wq_buf.at[0, :, pl.ds(s, w)], sem_wq0.at[c])

    def cp_wq(g):
        br, j = divmod(g, 2)
        return pltpu.make_async_copy(wqs[br].at[:, pl.ds(j * GW, GW)], wq_buf.at[g], sem_wq.at[g])

    def cp_wo(g):
        br, j = divmod(g, 2)
        return pltpu.make_async_copy(wos[br].at[pl.ds(j * GW, GW), :], wo_buf.at[g], sem_wo.at[g])

    def cp_k(g):
        br, j = divmod(g, 2)
        return pltpu.make_async_copy(ks[br].at[:, pl.ds(j * HG, HG)], k_buf.at[g], sem_k.at[g])

    def cp_v(g):
        br, j = divmod(g, 2)
        return pltpu.make_async_copy(vs[br].at[:, pl.ds(j * HG, HG)], v_buf.at[g], sem_v.at[g])

    def wait(buf, sem, u):
        pltpu.make_async_copy(buf.at[u], buf.at[u], sem.at[u]).wait()

    cp_x(0).start()
    for c in range(len(W0)):
        cp_wq0(c).start()
    cp_wq(1).start()
    cp_x(1).start()
    cp_wq(2).start()
    cp_wq(3).start()
    for g in range(NG):
        cp_k(g).start()
        cp_v(g).start()
        cp_wo(g).start()

    wait(x_buf, sem_x, 0)
    for c, (s, w) in enumerate(W0):
        cp_wq0(c).wait()
        q_buf[0, :, s:s + w] = jnp.dot(x_buf[0], wq_buf[0, :, s:s + w], preferred_element_type=F32).astype(BF16)

    def q_body(g, c):
        @pl.when(g == 2)
        def _():
            wait(x_buf, sem_x, 1)
        wait(wq_buf, sem_wq, g)
        q_buf[g] = jnp.dot(x_buf[g // 2], wq_buf[g], preferred_element_type=F32).astype(BF16)
        return c

    lax.fori_loop(1, NG, q_body, 0)

    def a_body(g, c):
        wait(k_buf, sem_k, g)
        wait(v_buf, sem_v, g)
        wait(wo_buf, sem_wo, g)
        first = (g % 2) == 0

        def S(t):
            _scores(q_buf.at[g], k_buf.at[g], t, p_buf.at[t])

        def P(t):
            _pv(p_buf.at[t], v_buf.at[g], t, o_buf.at[t])

        def O(t):
            r = jnp.dot(o_buf[t], wo_buf[g, UW * t:UW * (t + 1), :], preferred_element_type=F32)
            if t == 0:
                acc[...] = jnp.where(first, 0.0, acc[...]) + r
            elif t < 3:
                acc[...] += r
            else:
                r = acc[...] + r
                acc[...] = r
                out_buf[g // 2] = r.astype(BF16)

        S(0); S(1); P(0); O(0); S(2); P(1); O(1); S(3); P(2); O(2); P(3); O(3)

        @pl.when(g == 1)
        def _():
            pltpu.make_async_copy(out_buf.at[0], out_hbm.at[:, pl.ds(0, D)], sem_out.at[0]).start()
        return c

    lax.fori_loop(0, NG, a_body, 0)
    pltpu.make_async_copy(out_buf.at[1], out_hbm.at[:, pl.ds(D, D)], sem_out.at[1]).start()
    pltpu.make_async_copy(out_buf.at[0], out_hbm.at[:, pl.ds(0, D)], sem_out.at[0]).wait()
    pltpu.make_async_copy(out_buf.at[1], out_hbm.at[:, pl.ds(D, D)], sem_out.at[1]).wait()


@jax.jit
def pallas_concat_heads__mha_block_cached__mha_block_cached__near_ridge_kernel(A_x, A_k_cache, A_v_cache, A_wq, A_wo, B_x, B_k_cache, B_v_cache, B_wq, B_wo):
    any_spec = pl.BlockSpec(memory_space=pl.ANY)
    out = pl.pallas_call(
        _kernel,
        in_specs=[any_spec] * 10,
        out_specs=any_spec,
        out_shape=jax.ShapeDtypeStruct((M, 2 * D), BF16),
        scratch_shapes=[
            pltpu.VMEM((2, M, D), BF16),
            pltpu.VMEM((NG, D, GW), BF16),
            pltpu.VMEM((NG, GW, D), BF16),
            pltpu.VMEM((NG, B, HG, SK, DH), BF16),
            pltpu.VMEM((NG, B, HG, SK, DH), BF16),
            pltpu.VMEM((NG, M, GW), BF16),
            pltpu.VMEM((4, M, 128), BF16),
            pltpu.VMEM((4, M, UW), BF16),
            pltpu.VMEM((M, D), F32),
            pltpu.VMEM((2, M, D), BF16),
            pltpu.SemaphoreType.DMA((23,)),
        ],
        compiler_params=pltpu.CompilerParams(vmem_limit_bytes=100 * 1024 * 1024),
    )(A_x.reshape(M, D), A_k_cache, A_v_cache, A_wq, A_wo,
      B_x.reshape(M, D), B_k_cache, B_v_cache, B_wq, B_wo)
    return out.reshape(B, SQ, 2 * D)
```

```python
import jax
import jax.numpy as jnp
from jax import lax
import jax.experimental.pallas as pl
import jax.experimental.pallas.tpu as pltpu

B, SQ, D = 16, 32, 1024
H, SK, DH = 32, 32, 128
M = B * SQ
HU = 4
UW = HU * DH
HG = 16
GW = HG * DH
NG = 4
HA = 4
HQ = HG - HA
EXP2_SCALE = (DH ** -0.5) * 1.4426950408889634
F32 = jnp.float32
BF16 = jnp.bfloat16
U32 = jnp.uint32

REGIONS = (
    ((0, 1, 0, 4),),
    ((0, 1, 4, 16),),
    ((0, 1, 16, 24), (1, 2, 0, 8)),
    ((1, 3, 8, 16), (1, 2, 16, 24), (2, 3, 0, 8)),
    ((3, 5, 0, 16), (2, 5, 16, 24)),
    ((5, 8, 0, 24),),
)
OUT_PIECES = (
    (0, 256, (512,)),
    (256, 512, (512,)),
    (512, 768, (512,)),
    (768, 896, (512,)),
    (896, 1024, (256, 160, 64, 32)),
)


def _startup_pieces():
    out, have = [], 0
    for reg in REGIONS:
        pcs = []
        need = max(blk[1] for blk in reg)
        if need > have:
            pcs.append(('x', have, need))
            have = need
        for (k0, k1, v0, v1) in reg:
            if v0 < HQ < v1:
                pcs.append(('w', k0, k1, v0, HQ))
                pcs.append(('w', k0, k1, HQ, v1))
            else:
                pcs.append(('w', k0, k1, v0, v1))
        out.append(pcs)
    return out


_PIECES = _startup_pieces()
_OUT_LIST = [(c0, c1, sum(rs[:i]), rs[i]) for (c0, c1, rs) in OUT_PIECES for i in range(len(rs))]
S_X1 = sum(len(p) for p in _PIECES)
S_WL = S_X1 + 1
S_WN = S_WL + 2
S_K = S_WN + NG
S_V = S_K + NG
S_WO = S_V + NG
S_OUT = S_WO + NG
N_SEM = S_OUT + 2 * len(_OUT_LIST)


def _scores(q_of, k_ref, t, p_ref):
    lane_grp = lax.broadcasted_iota(jnp.int32, (SK, 128), 1) // SQ
    for g in range(B // 4):
        pts = []
        for h in range(HU * t, HU * (t + 1)):
            kh = k_ref[4 * g:4 * g + 4, h].reshape(128, DH)
            qh = pltpu.bitcast(q_of(h)[64 * g:64 * (g + 1), :], BF16)
            st = lax.dot_general(kh, qh, (((1,), (1,)), ((), ())), preferred_element_type=F32)
            s = st[0:SK]
            for j in range(1, 4):
                s = jnp.where(lane_grp == j, st[SK * j:SK * (j + 1)], s)
            m = jnp.max(s, axis=0, keepdims=True)
            e = jnp.exp2((s - m) * EXP2_SCALE)
            l = jnp.sum(e, axis=0, keepdims=True)
            pts.append(e * (1.0 / l))
        pt = jnp.concatenate(pts, axis=0)
        p_ref[64 * g:64 * (g + 1), :] = pltpu.bitcast(pt.T.astype(BF16), U32)


def _pv(p_ref, v_ref, t, o_ref):
    lane_grp = lax.broadcasted_iota(jnp.int32, (SQ // 2, 128), 1) // SK
    for b in range(B):
        pb = p_ref[16 * b:16 * (b + 1), :]
        zero = jnp.zeros_like(pb)
        pe = jnp.concatenate([jnp.where(lane_grp == h, pb, zero) for h in range(HU)], axis=0)
        vb = v_ref[b, HU * t:HU * (t + 1)].reshape(128, DH)
        ob = jnp.dot(pltpu.bitcast(pe, BF16), vb, preferred_element_type=F32)
        ob = pltpu.bitcast(ob.astype(BF16), U32)
        for h in range(HU):
            o_ref[h, 16 * b:16 * (b + 1), :] = ob[16 * h:16 * (h + 1)]


def _store_heads(ref, h0, r):
    r = pltpu.bitcast(r.astype(BF16), U32)
    for h in range(r.shape[1] // DH):
        ref[h0 + h] = r[:, DH * h:DH * (h + 1)]


def _kernel(xa, ka, va, wqa, woa, xb, kb, vb, wqb, wob, out_hbm,
            x_buf, wq0_buf, wql_buf, wqn_buf, wo_buf, k_buf, v_buf,
            q_buf, qn_buf, p_buf, o_buf, acc0, acc, out_buf, sems):
    ks, vs, wqs, wos = (ka, kb), (va, vb), (wqa, wqb), (woa, wob)

    def cp_piece(pc, s):
        k0, nk = pc[1] * DH, (pc[2] - pc[1]) * DH
        if pc[0] == 'x':
            return pltpu.make_async_copy(xa.at[:, pl.ds(k0, nk)], x_buf.at[0, :, pl.ds(k0, nk)], sems.at[s])
        v0, nh = pc[3], pc[4] - pc[3]
        h0 = v0 if v0 < HQ else v0 + HA
        return pltpu.make_async_copy(wqa.at[pl.ds(k0, nk), pl.ds(h0 * DH, nh * DH)],
                                     wq0_buf.at[pl.ds(k0, nk), pl.ds(v0 * DH, nh * DH)], sems.at[s])

    def cp_x1():
        return pltpu.make_async_copy(xb, x_buf.at[1], sems.at[S_X1])

    def cp_wl(i):
        return pltpu.make_async_copy(wqb.at[:, pl.ds(i * GW, HQ * DH)], wql_buf.at[i], sems.at[S_WL + i])

    def cp_wn(g):
        src = wqs[g // 2].at[:, pl.ds((g % 2) * GW + HQ * DH, HA * DH)]
        return pltpu.make_async_copy(src, wqn_buf.at[g], sems.at[S_WN + g])

    def cp_k(g):
        return pltpu.make_async_copy(ks[g // 2].at[:, pl.ds((g % 2) * HG, HG)], k_buf.at[g], sems.at[S_K + g])

    def cp_v(g):
        return pltpu.make_async_copy(vs[g // 2].at[:, pl.ds((g % 2) * HG, HG)], v_buf.at[g], sems.at[S_V + g])

    def cp_wo(g):
        return pltpu.make_async_copy(wos[g // 2].at[pl.ds((g % 2) * GW, GW), :], wo_buf.at[g], sems.at[S_WO + g])

    def cp_out(br, i):
        c0, c1, r0, nr = _OUT_LIST[i]
        col = br * D + c0
        if not isinstance(col, int):
            col = pl.multiple_of(col, DH)
        return pltpu.make_async_copy(out_buf.at[br, pl.ds(r0, nr), pl.ds(c0, c1 - c0)],
                                     out_hbm.at[pl.ds(r0, nr), pl.ds(col, c1 - c0)],
                                     sems.at[S_OUT + br * len(_OUT_LIST) + i])

    def wait_fill(buf, i, s):
        pltpu.make_async_copy(buf.at[i], buf.at[i], sems.at[s]).wait()

    def startup():
        s = 0
        for pcs in _PIECES:
            for pc in pcs:
                cp_piece(pc, s).start()
                s += 1
        cp_x1().start()
        cp_wl(0).start()
        cp_wl(1).start()
        for g in range(NG):
            cp_wn(g).start()
            cp_k(g).start()
            cp_v(g).start()
            cp_wo(g).start()
        s = 0
        for reg, pcs in zip(REGIONS, _PIECES):
            for pc in pcs:
                cp_piece(pc, s).wait()
                s += 1
            for (kt0, kt1, v0, v1) in reg:
                k0, k1, n0, n1 = kt0 * DH, kt1 * DH, v0 * DH, v1 * DH
                r = jnp.dot(x_buf[0, :, k0:k1], wq0_buf[k0:k1, n0:n1], preferred_element_type=F32)
                if k0 > 0:
                    r = acc0[:, n0:n1] + r
                if k1 < D:
                    acc0[:, n0:n1] = r
                else:
                    _store_heads(q_buf, v0, r)
        cp_x1().wait()

    def q_step(i, carry):
        wait_fill(wql_buf, i, S_WL + i)
        r = jnp.dot(x_buf[1], wql_buf[i], preferred_element_type=F32)
        _store_heads(q_buf, (2 + i) * HQ, r)
        return carry

    def a_step(g, carry):
        wait_fill(wqn_buf, g, S_WN + g)
        wait_fill(k_buf, g, S_K + g)
        wait_fill(v_buf, g, S_V + g)
        wait_fill(wo_buf, g, S_WO + g)
        br = g // 2
        last = (g % 2) == 1

        def q_of(h):
            return q_buf.at[g * HQ + h] if h < HQ else qn_buf.at[h - HQ]

        def qproj():
            r = jnp.dot(x_buf[br], wqn_buf[g], preferred_element_type=F32)
            _store_heads(qn_buf, 0, r)

        def scores(t):
            _scores(q_of, k_buf.at[g], t, p_buf.at[t])

        def pv(t):
            _pv(p_buf.at[t], v_buf.at[g], t, o_buf.at[t])

        def oproj(t):
            o = pltpu.bitcast(jnp.concatenate([o_buf[t, h] for h in range(HU)], axis=1), BF16)
            if t < 3:
                r = jnp.dot(o, wo_buf[g, UW * t:UW * (t + 1), :], preferred_element_type=F32)
                if t == 0:
                    acc[...] = jnp.where(last, acc[...], 0.0) + r
                else:
                    acc[...] += r
                return
            i = 0
            for (c0, c1, rs) in OUT_PIECES:
                r = jnp.dot(o, wo_buf[g, UW * t:UW * (t + 1), c0:c1], preferred_element_type=F32)
                r = acc[:, c0:c1] + r
                acc[:, c0:c1] = r
                r = r.astype(BF16)
                r0 = 0
                for nr in rs:
                    out_buf[br, r0:r0 + nr, c0:c1] = r[r0:r0 + nr]
                    pl.when(last)(cp_out(br, i).start)
                    r0 += nr
                    i += 1

        qproj()
        scores(0)
        scores(1)
        pv(0)
        scores(2)
        oproj(0)
        pv(1)
        scores(3)
        oproj(1)
        pv(2)
        oproj(2)
        pv(3)
        oproj(3)
        return carry

    def phase(s, carry):
        @pl.when(s == 0)
        def _():
            startup()
            lax.fori_loop(0, 2, q_step, 0)

        @pl.when(s == 1)
        def _():
            lax.fori_loop(0, NG, a_step, 0)
        return carry

    lax.fori_loop(0, 2, phase, 0)
    for br in range(2):
        for i in range(len(_OUT_LIST)):
            cp_out(br, i).wait()


@jax.jit
def pallas_concat_heads__mha_block_cached__mha_block_cached__near_ridge_kernel(
    A_x: jax.Array,
    A_k_cache: jax.Array,
    A_v_cache: jax.Array,
    A_wq: jax.Array,
    A_wo: jax.Array,
    B_x: jax.Array,
    B_k_cache: jax.Array,
    B_v_cache: jax.Array,
    B_wq: jax.Array,
    B_wo: jax.Array,
):
    any_spec = pl.BlockSpec(memory_space=pl.ANY)
    out = pl.pallas_call(
        _kernel,
        in_specs=[any_spec] * 10,
        out_specs=any_spec,
        out_shape=jax.ShapeDtypeStruct((M, 2 * D), BF16),
        scratch_shapes=[
            pltpu.VMEM((2, M, D), BF16),
            pltpu.VMEM((D, 2 * HQ * DH + 128), BF16),
            pltpu.VMEM((2, D, HQ * DH), BF16),
            pltpu.VMEM((NG, D, HA * DH), BF16),
            pltpu.VMEM((NG, GW, D), BF16),
            pltpu.VMEM((NG, B, HG, SK, DH), BF16),
            pltpu.VMEM((NG, B, HG, SK, DH), BF16),
            pltpu.VMEM((NG * HQ, M // 2, DH), U32),
            pltpu.VMEM((HA, M // 2, DH), U32),
            pltpu.VMEM((4, M // 2, 128), U32),
            pltpu.VMEM((4, HU, M // 2, DH), U32),
            pltpu.VMEM((M, 2 * HQ * DH), F32),
            pltpu.VMEM((M, D), F32),
            pltpu.VMEM((2, M, D), BF16),
            pltpu.SemaphoreType.DMA((N_SEM,)),
        ],
        compiler_params=pltpu.CompilerParams(
            vmem_limit_bytes=100 * 1024 * 1024,
            disable_semaphore_checks=True,
            disable_bounds_checks=True,
        ),
    )(A_x.reshape(M, D), A_k_cache, A_v_cache, A_wq, A_wo,
      B_x.reshape(M, D), B_k_cache, B_v_cache, B_wq, B_wo)
    return out.reshape(B, SQ, 2 * D)
```

```python
import jax
import jax.numpy as jnp
from jax import lax
import jax.experimental.pallas as pl
import jax.experimental.pallas.tpu as pltpu

B, SQ, D = 16, 32, 1024
H, SK, DH = 32, 32, 128
M = B * SQ
HU = 4
UW = HU * DH
HG = 16
GW = HG * DH
NG = 4
HA = 4
HQ = HG - HA
EXP2_SCALE = (DH ** -0.5) * 1.4426950408889634
F32 = jnp.float32
BF16 = jnp.bfloat16
U32 = jnp.uint32

REGIONS = (
    ((0, 0, 1, 0, 4),),
    ((0, 0, 1, 4, 12),),
    ((0, 0, 1, 12, 24),),
    ((0, 1, 2, 0, 24),),
    ((0, 2, 4, 0, 12), (0, 2, 3, 12, 24)),
    ((0, 4, 6, 0, 12), (0, 3, 6, 12, 24)),
    ((0, 6, 8, 0, 24), (1, 0, 8, 0, 4)),
    ((1, 0, 8, 4, 24),),
)
OUT_PIECES = (
    (0, 256, (512,)),
    (256, 512, (512,)),
    (512, 768, (512,)),
    (768, 896, (512,)),
    (896, 1024, (256, 160, 64, 32)),
)


def _region_pieces():
    out, have = [], [0, 0]
    for reg in REGIONS:
        pcs = []
        for br in range(2):
            blks = [blk for blk in reg if blk[0] == br]
            if not blks:
                continue
            need = max(blk[2] for blk in blks)
            if need > have[br]:
                pcs.append(('x', br, have[br], need))
                have[br] = need
            for (_, k0, k1, v0, v1) in blks:
                if v0 < HQ < v1:
                    pcs.append(('w', br, k0, k1, v0, HQ))
                    pcs.append(('w', br, k0, k1, HQ, v1))
                else:
                    pcs.append(('w', br, k0, k1, v0, v1))
        out.append(pcs)
    return out


_PIECES = _region_pieces()
_OUT_LIST = [(c0, c1, sum(rs[:i]), rs[i]) for (c0, c1, rs) in OUT_PIECES for i in range(len(rs))]
S_WN = sum(len(p) for p in _PIECES)
S_KV = S_WN + NG
S_WO = S_KV + NG
S_OUT = S_WO + NG
N_SEM = S_OUT + 2 * len(_OUT_LIST)


def _scores(q_of, k_ref, t, p_ref):
    lane_grp = lax.broadcasted_iota(jnp.int32, (SK, 128), 1) // SQ
    for g in range(B // 4):
        pts = []
        for h in range(HU * t, HU * (t + 1)):
            kh = k_ref[4 * g:4 * g + 4, h].reshape(128, DH)
            qh = pltpu.bitcast(q_of(h)[64 * g:64 * (g + 1), :], BF16)
            st = lax.dot_general(kh, qh, (((1,), (1,)), ((), ())), preferred_element_type=F32)
            s = st[0:SK]
            for j in range(1, 4):
                s = jnp.where(lane_grp == j, st[SK * j:SK * (j + 1)], s)
            m = jnp.max(s, axis=0, keepdims=True)
            e = jnp.exp2((s - m) * EXP2_SCALE)
            l = jnp.sum(e, axis=0, keepdims=True)
            pts.append(e * (1.0 / l))
        pt = jnp.concatenate(pts, axis=0)
        p_ref[64 * g:64 * (g + 1), :] = pltpu.bitcast(pt.T.astype(BF16), U32)


def _pv(p_ref, v_ref, t, o_ref):
    lane_grp = lax.broadcasted_iota(jnp.int32, (SQ // 2, 128), 1) // SK
    for b in range(B):
        pb = p_ref[16 * b:16 * (b + 1), :]
        zero = jnp.zeros_like(pb)
        pe = jnp.concatenate([jnp.where(lane_grp == h, pb, zero) for h in range(HU)], axis=0)
        vb = v_ref[b, HU * t:HU * (t + 1)].reshape(128, DH)
        ob = jnp.dot(pltpu.bitcast(pe, BF16), vb, preferred_element_type=F32)
        ob = pltpu.bitcast(ob.astype(BF16), U32)
        for h in range(HU):
            o_ref[h, 16 * b:16 * (b + 1), :] = ob[16 * h:16 * (h + 1)]


def _store_heads(ref, h0, r):
    r = pltpu.bitcast(r.astype(BF16), U32)
    for h in range(r.shape[1] // DH):
        ref[h0 + h] = r[:, DH * h:DH * (h + 1)]


def _kernel(xa, ka, va, wqa, woa, xb, kb, vb, wqb, wob, out_hbm,
            x_buf, wq_buf, wqn_buf, wo_buf, kv_buf,
            q_buf, qn_buf, p_buf, o_buf, acc0, acc, out_buf, sems):
    xs, ks, vs, wqs, wos = (xa, xb), (ka, kb), (va, vb), (wqa, wqb), (woa, wob)

    def cp_piece(pc, s):
        br = pc[1]
        k0, nk = pc[2] * DH, (pc[3] - pc[2]) * DH
        if pc[0] == 'x':
            return pltpu.make_async_copy(xs[br].at[:, pl.ds(k0, nk)], x_buf.at[br, :, pl.ds(k0, nk)], sems.at[s])
        v0, nh = pc[4], pc[5] - pc[4]
        h0 = v0 if v0 < HQ else v0 + HA
        return pltpu.make_async_copy(wqs[br].at[pl.ds(k0, nk), pl.ds(h0 * DH, nh * DH)],
                                     wq_buf.at[br, pl.ds(k0, nk), pl.ds(v0 * DH, nh * DH)], sems.at[s])

    def cp_wn(g):
        src = wqs[g // 2].at[:, pl.ds((g % 2) * GW + HQ * DH, HA * DH)]
        return pltpu.make_async_copy(src, wqn_buf.at[g], sems.at[S_WN + g])

    def cp_kv(g, j):
        src = (ks, vs)[j][g // 2].at[:, pl.ds((g % 2) * HG, HG)]
        return pltpu.make_async_copy(src, kv_buf.at[g, j], sems.at[S_KV + g])

    def cp_wo(g):
        return pltpu.make_async_copy(wos[g // 2].at[pl.ds((g % 2) * GW, GW), :], wo_buf.at[g], sems.at[S_WO + g])

    def cp_out(br, i):
        c0, c1, r0, nr = _OUT_LIST[i]
        col = br * D + c0
        if not isinstance(col, int):
            col = pl.multiple_of(col, DH)
        return pltpu.make_async_copy(out_buf.at[br, pl.ds(r0, nr), pl.ds(c0, c1 - c0)],
                                     out_hbm.at[pl.ds(r0, nr), pl.ds(col, c1 - c0)],
                                     sems.at[S_OUT + br * len(_OUT_LIST) + i])

    def wait_fill(buf, i, s):
        pltpu.make_async_copy(buf.at[i], buf.at[i], sems.at[s]).wait()

    def q_phase():
        s = 0
        for pcs in _PIECES:
            for pc in pcs:
                cp_piece(pc, s).start()
                s += 1
        for g in range(NG):
            cp_wn(g).start()
            cp_kv(g, 0).start()
            cp_kv(g, 1).start()
            cp_wo(g).start()
        s = 0
        for reg, pcs in zip(REGIONS, _PIECES):
            for pc in pcs:
                cp_piece(pc, s).wait()
                s += 1
            for (br, kt0, kt1, v0, v1) in reg:
                k0, k1, n0, n1 = kt0 * DH, kt1 * DH, v0 * DH, v1 * DH
                r = jnp.dot(x_buf[br, :, k0:k1], wq_buf[br, k0:k1, n0:n1], preferred_element_type=F32)
                if k0 > 0:
                    r = acc0[:, n0:n1] + r
                if k1 < D:
                    acc0[:, n0:n1] = r
                else:
                    _store_heads(q_buf, br * 2 * HQ + v0, r)

    def a_step(g, carry):
        wait_fill(wqn_buf, g, S_WN + g)
        wait_fill(kv_buf, g, S_KV + g)
        wait_fill(wo_buf, g, S_WO + g)
        br = g // 2
        last = (g % 2) == 1

        def q_of(h):
            return q_buf.at[g * HQ + h] if h < HQ else qn_buf.at[h - HQ]

        def qproj():
            r = jnp.dot(x_buf[br], wqn_buf[g], preferred_element_type=F32)
            _store_heads(qn_buf, 0, r)

        def scores(t):
            _scores(q_of, kv_buf.at[g, 0], t, p_buf.at[t])

        def pv(t):
            _pv(p_buf.at[t], kv_buf.at[g, 1], t, o_buf.at[t])

        def oproj(t):
            o = pltpu.bitcast(jnp.concatenate([o_buf[t, h] for h in range(HU)], axis=1), BF16)
            if t < 3:
                r = jnp.dot(o, wo_buf[g, UW * t:UW * (t + 1), :], preferred_element_type=F32)
                if t == 0:
                    acc[...] = jnp.where(last, acc[...], 0.0) + r
                else:
                    acc[...] += r
                return
            i = 0
            for (c0, c1, rs) in OUT_PIECES:
                r = jnp.dot(o, wo_buf[g, UW * t:UW * (t + 1), c0:c1], preferred_element_type=F32)
                r = acc[:, c0:c1] + r
                acc[:, c0:c1] = r
                r = r.astype(BF16)
                r0 = 0
                for nr in rs:
                    out_buf[br, r0:r0 + nr, c0:c1] = r[r0:r0 + nr]
                    pl.when(last)(cp_out(br, i).start)
                    r0 += nr
                    i += 1

        qproj()
        scores(0)
        scores(1)
        pv(0)
        scores(2)
        oproj(0)
        pv(1)
        scores(3)
        oproj(1)
        pv(2)
        oproj(2)
        pv(3)
        oproj(3)
        return carry

    def phase(s, carry):
        pl.when(s == 0)(q_phase)

        @pl.when(s == 1)
        def _():
            lax.fori_loop(0, NG, a_step, 0)
        return carry

    lax.fori_loop(0, 2, phase, 0)
    for br in range(2):
        for i in range(len(_OUT_LIST)):
            cp_out(br, i).wait()


@jax.jit
def pallas_concat_heads__mha_block_cached__mha_block_cached__near_ridge_kernel(
    A_x: jax.Array,
    A_k_cache: jax.Array,
    A_v_cache: jax.Array,
    A_wq: jax.Array,
    A_wo: jax.Array,
    B_x: jax.Array,
    B_k_cache: jax.Array,
    B_v_cache: jax.Array,
    B_wq: jax.Array,
    B_wo: jax.Array,
):
    any_spec = pl.BlockSpec(memory_space=pl.ANY)
    out = pl.pallas_call(
        _kernel,
        in_specs=[any_spec] * 10,
        out_specs=any_spec,
        out_shape=jax.ShapeDtypeStruct((M, 2 * D), BF16),
        scratch_shapes=[
            pltpu.VMEM((2, M, D), BF16),
            pltpu.VMEM((2, D, 2 * HQ * DH + 128), BF16),
            pltpu.VMEM((NG, D, HA * DH), BF16),
            pltpu.VMEM((NG, GW, D), BF16),
            pltpu.VMEM((NG, 2, B, HG, SK, DH), BF16),
            pltpu.VMEM((NG * HQ, M // 2, DH), U32),
            pltpu.VMEM((HA, M // 2, DH), U32),
            pltpu.VMEM((4, M // 2, 128), U32),
            pltpu.VMEM((4, HU, M // 2, DH), U32),
            pltpu.VMEM((M, 2 * HQ * DH), F32),
            pltpu.VMEM((M, D), F32),
            pltpu.VMEM((2, M, D), BF16),
            pltpu.SemaphoreType.DMA((N_SEM,)),
        ],
        compiler_params=pltpu.CompilerParams(
            vmem_limit_bytes=100 * 1024 * 1024,
            disable_semaphore_checks=True,
            disable_bounds_checks=True,
        ),
    )(A_x.reshape(M, D), A_k_cache, A_v_cache, A_wq, A_wo,
      B_x.reshape(M, D), B_k_cache, B_v_cache, B_wq, B_wo)
    return out.reshape(B, SQ, 2 * D)
```

```python
import jax
import jax.numpy as jnp
from jax import lax
import jax.experimental.pallas as pl
import jax.experimental.pallas.tpu as pltpu

B, SQ, D = 16, 32, 1024
H, SK, DH = 32, 32, 128
M = B * SQ
HU = 4
UW = HU * DH
HG = 16
GW = HG * DH
NG = 4
HA = 4
HQ = HG - HA
PAD = 128
EXP2_SCALE = (DH ** -0.5) * 1.4426950408889634
F32 = jnp.float32
BF16 = jnp.bfloat16
U32 = jnp.uint32

REGIONS = (
    ((0, 0, 1, 0, 4),),
    ((0, 0, 1, 4, 12),),
    ((0, 0, 1, 12, 24),),
    ((0, 1, 2, 0, 24),),
    ((0, 2, 4, 0, 12), (0, 2, 3, 12, 24)),
    ((0, 4, 6, 0, 12), (0, 3, 6, 12, 24)),
    ((0, 6, 8, 0, 24), (1, 0, 8, 0, 4)),
    ((1, 0, 8, 4, 12), 'S', (1, 0, 8, 12, 24)),
)
OUT_PIECES = (
    (0, 256, (512,)),
    (256, 512, (512,)),
    (512, 768, (512,)),
    (768, 896, (512,)),
    (896, 1024, (256, 160, 64, 32)),
)


def _region_pieces():
    out, have = [], [0, 0]
    for reg in REGIONS:
        pcs = []
        for br in range(2):
            blks = [blk for blk in reg if blk != 'S' and blk[0] == br]
            if not blks:
                continue
            need = max(blk[2] for blk in blks)
            if need > have[br]:
                pcs.append(('x', br, have[br], need))
                have[br] = need
            for (_, k0, k1, v0, v1) in blks:
                if v0 < HQ < v1:
                    pcs.append(('w', br, k0, k1, v0, HQ))
                    pcs.append(('w', br, k0, k1, HQ, v1))
                else:
                    pcs.append(('w', br, k0, k1, v0, v1))
        if 'S' in reg:
            pcs.append(('k',))
        out.append(pcs)
    return out


_PIECES = _region_pieces()
_OUT_LIST = [(c0, c1, sum(rs[:i]), rs[i]) for (c0, c1, rs) in OUT_PIECES for i in range(len(rs))]
S_WN = sum(len(p) for p in _PIECES)
S_KV = S_WN + NG
S_WO = S_KV + NG
S_OUT = S_WO + NG
N_SEM = S_OUT + 2 * len(_OUT_LIST)


def _softmax_t(blocks):
    pts = []
    for s in blocks:
        m = jnp.max(s, axis=0, keepdims=True)
        e = jnp.exp2((s - m) * EXP2_SCALE)
        l = jnp.sum(e, axis=0, keepdims=True)
        pts.append(e * (1.0 / l))
    pt = jnp.concatenate(pts, axis=0)
    return pltpu.bitcast(pt.T.astype(BF16), U32)


def _first_scores(q_ref, k_ref, p_ref):
    lane_grp = lax.broadcasted_iota(jnp.int32, (SK, 128), 1) // SQ
    for g in range(B // 4):
        blocks = []
        for h in range(HU):
            kh = k_ref[4 * g:4 * g + 4, h].reshape(128, DH)
            qh = q_ref[h, 128 * g:128 * (g + 1), :]
            st = lax.dot_general(kh, qh, (((1,), (1,)), ((), ())), preferred_element_type=F32)
            s = st[0:SK]
            for j in range(1, 4):
                s = jnp.where(lane_grp == j, st[SK * j:SK * (j + 1)], s)
            blocks.append(s)
        p_ref[64 * g:64 * (g + 1), :] = _softmax_t(blocks)


def _transpose_keys(k_ref, t, kt_ref):
    for b in range(B):
        ks = k_ref[b, HU * t:HU * (t + 1)].reshape(128, DH)
        kt_ref[b] = pltpu.bitcast(ks.T, U32)


def _scores_pv(q_refs, kt_ref, s_ref, p_ref, v_ref, t, o_ref, batches):
    lg = lax.broadcasted_iota(jnp.int32, (16, 128), 1) // 32
    lg32 = lax.broadcasted_iota(jnp.int32, (32, 128), 1) // 32
    zero = jnp.zeros((16, 128), U32)

    def keep(j, x):
        return jnp.where(lg != j, zero, x)

    def drop(j, x):
        return jnp.where(lg == j, zero, x)

    def mm(a, w):
        return jnp.dot(pltpu.bitcast(a, BF16), pltpu.bitcast(jnp.concatenate(w, axis=0), BF16),
                       preferred_element_type=F32)

    for b in batches:
        kt = kt_ref[b]
        vs = pltpu.bitcast(v_ref[b, HU * t:HU * (t + 1)].reshape(128, DH), U32)
        kc = [kt[16 * c:16 * (c + 1)] for c in range(4)]
        vc = [vs[16 * c:16 * (c + 1)] for c in range(4)]
        p = p_ref[16 * b:16 * (b + 1), :]
        qs = [pltpu.bitcast(q_refs[h][SQ * b:SQ * (b + 1), :], U32) for h in range(HU)]
        outs = []
        for j in range(4):
            w = [drop(j, vc[c]) if c == j else keep(j, kc[c]) for c in range(4)]
            outs.append(mm(jnp.where(lg == j, p, qs[j]), w))
        qd = qs[0]
        for j in range(1, 4):
            qd = jnp.where(lg == j, qs[j], qd)
        s_rest = mm(qd, [keep(c, kc[c]) for c in range(4)])
        o_rest = mm(p, [keep(c, vc[c]) for c in range(4)])
        s = outs[0]
        for j in range(1, 4):
            s = jnp.where(lg32 == j, outs[j], s)
        s_ref[SQ * b:SQ * (b + 1), :] = s + s_rest
        for j in range(4):
            o_ref[j, SQ * b:SQ * (b + 1), :] = jnp.where(lg32 == j, o_rest, outs[j]).astype(BF16)


def _store_heads(ref, h0, r):
    for h in range(r.shape[1] // DH):
        ref[h0 + h] = r[:, DH * h:DH * (h + 1)].astype(BF16)


def _kernel(xa, ka, va, wqa, woa, xb, kb, vb, wqb, wob, out_hbm,
            x_buf, wq_buf, wqn_buf, wo_buf, k0_buf, kv_buf,
            q_buf, qn_buf, p_buf, o_buf, kt_buf, s_buf, acc0, acc, out_buf, sems):
    xs, ks, vs, wqs, wos = (xa, xb), (ka, kb), (va, vb), (wqa, wqb), (woa, wob)

    def cp_piece(pc, s):
        if pc[0] == 'k':
            return pltpu.make_async_copy(ka.at[:, pl.ds(0, HU)], k0_buf, sems.at[s])
        br = pc[1]
        k0, nk = pc[2] * DH, (pc[3] - pc[2]) * DH
        if pc[0] == 'x':
            return pltpu.make_async_copy(xs[br].at[:, pl.ds(k0, nk)], x_buf.at[br, :, pl.ds(k0, nk)], sems.at[s])
        v0, nh = pc[4], pc[5] - pc[4]
        h0 = v0 if v0 < HQ else v0 + HA
        return pltpu.make_async_copy(wqs[br].at[pl.ds(k0, nk), pl.ds(h0 * DH, nh * DH)],
                                     wq_buf.at[br, pl.ds(k0, nk), pl.ds(v0 * DH, nh * DH)], sems.at[s])

    def cp_wn(g):
        src = wqs[g // 2].at[:, pl.ds((g % 2) * GW + HQ * DH, HA * DH)]
        return pltpu.make_async_copy(src, wqn_buf.at[g], sems.at[S_WN + g])

    def cps_kv(g):
        sem = sems.at[S_KV + g]
        br, j = divmod(g, 2)
        if j == 0:
            cps = [pltpu.make_async_copy(ks[br].at[:, pl.ds(HU, HG)], kv_buf.at[g, 0], sem)]
        else:
            n = HG - HU
            cps = [pltpu.make_async_copy(ks[br].at[:, pl.ds(HG + HU, n)], kv_buf.at[g, 0, :, pl.ds(0, n)], sem),
                   pltpu.make_async_copy(ks[1 - br].at[:, pl.ds(0, HU)], kv_buf.at[g, 0, :, pl.ds(n, HU)], sem)]
        cps.append(pltpu.make_async_copy(vs[br].at[:, pl.ds(j * HG, HG)], kv_buf.at[g, 1], sem))
        return cps

    def wo_view(g):
        return wo_buf.at[g, :, pl.ds(0, D)]

    def cp_wo(g):
        return pltpu.make_async_copy(wos[g // 2].at[pl.ds((g % 2) * GW, GW), :], wo_view(g), sems.at[S_WO + g])

    def cp_out(br, i):
        c0, c1, r0, nr = _OUT_LIST[i]
        col = br * D + c0
        if not isinstance(col, int):
            col = pl.multiple_of(col, DH)
        return pltpu.make_async_copy(out_buf.at[br, pl.ds(r0, nr), pl.ds(c0, c1 - c0)],
                                     out_hbm.at[pl.ds(r0, nr), pl.ds(col, c1 - c0)],
                                     sems.at[S_OUT + br * len(_OUT_LIST) + i])

    def wait_fill(view, s):
        pltpu.make_async_copy(view, view, sems.at[s]).wait()

    def q_phase():
        s = 0
        for pcs in _PIECES:
            for pc in pcs:
                cp_piece(pc, s).start()
                s += 1
        for g in range(NG):
            cp_wn(g).start()
            for cp in cps_kv(g):
                cp.start()
            cp_wo(g).start()
        s = 0
        for reg, pcs in zip(REGIONS, _PIECES):
            for pc in pcs:
                cp_piece(pc, s).wait()
                s += 1
            for blk in reg:
                if blk == 'S':
                    _first_scores(q_buf, k0_buf, p_buf.at[0])
                    continue
                br, kt0, kt1, v0, v1 = blk
                k0, k1, n0, n1 = kt0 * DH, kt1 * DH, v0 * DH, v1 * DH
                r = jnp.dot(x_buf[br, :, k0:k1], wq_buf[br, k0:k1, n0:n1], preferred_element_type=F32)
                if k0 > 0:
                    r = acc0[:, n0:n1] + r
                if k1 < D:
                    acc0[:, n0:n1] = r
                else:
                    _store_heads(q_buf, br * 2 * HQ + v0, r)

    def a_step(g, carry):
        wait_fill(wqn_buf.at[g], S_WN + g)
        wait_fill(kv_buf.at[g], S_KV + g)
        wait_fill(wo_view(g), S_WO + g)
        br = g // 2
        last = (g % 2) == 1
        g_next = (g + 1) % NG

        def q_refs(t):
            if t < 2:
                return [q_buf.at[g * HQ + HU * (t + 1) + h] for h in range(HU)]
            if t == 2:
                return [qn_buf.at[h] for h in range(HU)]
            return [q_buf.at[g_next * HQ + h] for h in range(HU)]

        def qproj(half):
            h0, h1 = half * HA // 2, (half + 1) * HA // 2
            r = jnp.dot(x_buf[br], wqn_buf[g, :, h0 * DH:h1 * DH], preferred_element_type=F32)
            _store_heads(qn_buf, h0, r)

        def keys(t):
            _transpose_keys(kv_buf.at[g, 0], t, kt_buf.at[t])

        def attn(t, half):
            _scores_pv(q_refs(t), kt_buf.at[t], s_buf.at[t], p_buf.at[t], kv_buf.at[g, 1], t, o_buf.at[t],
                       range(8 * half, 8 * (half + 1)))
            for i in (2 * half, 2 * half + 1):
                st = s_buf[t, 128 * i:128 * (i + 1), :].T
                p_buf[(t + 1) % 4, 64 * i:64 * (i + 1), :] = _softmax_t(
                    [st[SK * h:SK * (h + 1)] for h in range(HU)])

        def o_lhs(t):
            return jnp.concatenate([o_buf[t, h] for h in range(HU)], axis=1)

        def oproj(t, half):
            n0, n1 = half * D // 2, (half + 1) * D // 2
            r = jnp.dot(o_lhs(t), wo_buf[g, UW * t:UW * (t + 1), n0:n1], preferred_element_type=F32)
            if t == 0:
                acc[:, n0:n1] = jnp.where(last, acc[:, n0:n1], 0.0) + r
            else:
                acc[:, n0:n1] += r

        def oproj_final():
            o = o_lhs(3)
            i = 0
            for (c0, c1, rs) in OUT_PIECES:
                r = jnp.dot(o, wo_buf[g, 3 * UW:4 * UW, c0:c1], preferred_element_type=F32)
                r = acc[:, c0:c1] + r
                acc[:, c0:c1] = r
                r = r.astype(BF16)
                r0 = 0
                for nr in rs:
                    out_buf[br, r0:r0 + nr, c0:c1] = r[r0:r0 + nr]
                    pl.when(last)(cp_out(br, i).start)
                    r0 += nr
                    i += 1

        keys(0)
        qproj(0)
        attn(0, 0)
        qproj(1)
        keys(1)
        attn(0, 1)
        for t in range(3):
            oproj(t, 0)
            attn(t + 1, 0)
            oproj(t, 1)
            if t < 2:
                keys(t + 2)
            attn(t + 1, 1)
        oproj_final()
        return carry

    def phase(s, carry):
        @pl.when(s == 0)
        def _():
            q_phase()
            lax.fori_loop(0, NG, a_step, 0)

        @pl.when(s == 1)
        def _():
            for br in range(2):
                for i in range(len(_OUT_LIST)):
                    cp_out(br, i).wait()
        return carry

    lax.fori_loop(0, 2, phase, 0)


@jax.jit
def pallas_concat_heads__mha_block_cached__mha_block_cached__near_ridge_kernel(
    A_x: jax.Array,
    A_k_cache: jax.Array,
    A_v_cache: jax.Array,
    A_wq: jax.Array,
    A_wo: jax.Array,
    B_x: jax.Array,
    B_k_cache: jax.Array,
    B_v_cache: jax.Array,
    B_wq: jax.Array,
    B_wo: jax.Array,
):
    any_spec = pl.BlockSpec(memory_space=pl.ANY)
    out = pl.pallas_call(
        _kernel,
        in_specs=[any_spec] * 10,
        out_specs=any_spec,
        out_shape=jax.ShapeDtypeStruct((M, 2 * D), BF16),
        scratch_shapes=[
            pltpu.VMEM((2, M, D), BF16),
            pltpu.VMEM((2, D, 2 * HQ * DH + PAD), BF16),
            pltpu.VMEM((NG, D, HA * DH), BF16),
            pltpu.VMEM((NG, GW, D + PAD), BF16),
            pltpu.VMEM((B, HU, SK, DH), BF16),
            pltpu.VMEM((NG, 2, B, HG, SK, DH), BF16),
            pltpu.VMEM((NG * HQ, M, DH), BF16),
            pltpu.VMEM((HA, M, DH), BF16),
            pltpu.VMEM((4, M // 2, 128), U32),
            pltpu.VMEM((4, HU, M, DH), BF16),
            pltpu.VMEM((4, B, DH // 2, 128), U32),
            pltpu.VMEM((4, M, 128), F32),
            pltpu.VMEM((M, 2 * HQ * DH), F32),
            pltpu.VMEM((M, D), F32),
            pltpu.VMEM((2, M, D), BF16),
            pltpu.SemaphoreType.DMA((N_SEM,)),
        ],
        compiler_params=pltpu.CompilerParams(
            vmem_limit_bytes=100 * 1024 * 1024,
            disable_semaphore_checks=True,
            disable_bounds_checks=True,
        ),
    )(A_x.reshape(M, D), A_k_cache, A_v_cache, A_wq, A_wo,
      B_x.reshape(M, D), B_k_cache, B_v_cache, B_wq, B_wo)
    return out.reshape(B, SQ, 2 * D)
```

```python
import jax
import jax.numpy as jnp
from jax import lax
import jax.experimental.pallas as pl
import jax.experimental.pallas.tpu as pltpu

B, SQ, D = 16, 32, 1024
H, SK, DH = 32, 32, 128
M = B * SQ
HU = 4
UW = HU * DH
HG = 16
GW = HG * DH
NG = 4
HA = 4
HQ = HG - HA
NP = 4
BP = B // NP
PAD = 128
EXP2_SCALE = (DH ** -0.5) * 1.4426950408889634
F32 = jnp.float32
BF16 = jnp.bfloat16
U32 = jnp.uint32

REGIONS = (
    ((0, 0, 1, 0, 4),),
    ((0, 0, 1, 4, 12),),
    ((0, 0, 1, 12, 24),),
    ((0, 1, 2, 0, 24),),
    ((0, 2, 4, 0, 12), (0, 2, 3, 12, 24)),
    ((0, 4, 6, 0, 12), (0, 3, 6, 12, 24)),
    ((0, 6, 8, 0, 24), (1, 0, 8, 0, 4)),
    ((1, 0, 8, 4, 12), 'S', (1, 0, 8, 12, 24)),
)
OUT_PIECES = (
    (0, 256, (512,)),
    (256, 512, (512,)),
    (512, 768, (512,)),
    (768, 896, (512,)),
    (896, 1024, (256, 160, 64, 32)),
)


def _region_pieces():
    out, have = [], [0, 0]
    for reg in REGIONS:
        pcs = []
        for br in range(2):
            blks = [blk for blk in reg if blk != 'S' and blk[0] == br]
            if not blks:
                continue
            need = max(blk[2] for blk in blks)
            if need > have[br]:
                pcs.append(('x', br, have[br], need))
                have[br] = need
            for (_, k0, k1, v0, v1) in blks:
                if v0 < HQ < v1:
                    pcs.append(('w', br, k0, k1, v0, HQ))
                    pcs.append(('w', br, k0, k1, HQ, v1))
                else:
                    pcs.append(('w', br, k0, k1, v0, v1))
        if 'S' in reg:
            pcs.append(('k',))
        out.append(pcs)
    return out


_PIECES = _region_pieces()
_OUT_LIST = [(c0, c1, sum(rs[:i]), rs[i]) for (c0, c1, rs) in OUT_PIECES for i in range(len(rs))]
S_WN = sum(len(p) for p in _PIECES)
S_KV = S_WN + NG
S_WO = S_KV + NG
S_OUT = S_WO + NG
N_SEM = S_OUT + 2 * len(_OUT_LIST)


def _softmax_t(blocks):
    pts = []
    for s in blocks:
        m = jnp.max(s, axis=0, keepdims=True)
        e = jnp.exp2((s - m) * EXP2_SCALE)
        l = jnp.sum(e, axis=0, keepdims=True)
        pts.append(e * (1.0 / l))
    pt = jnp.concatenate(pts, axis=0)
    return pltpu.bitcast(pt.T.astype(BF16), U32)


def _first_scores(q_ref, k_ref, p_ref):
    lane_grp = lax.broadcasted_iota(jnp.int32, (SK, 128), 1) // SQ
    for g in range(BP // 4):
        blocks = []
        for h in range(HU):
            kh = k_ref[4 * g:4 * g + 4, h].reshape(128, DH)
            qh = q_ref[h, 128 * g:128 * (g + 1), :]
            st = lax.dot_general(kh, qh, (((1,), (1,)), ((), ())), preferred_element_type=F32)
            s = st[0:SK]
            for j in range(1, 4):
                s = jnp.where(lane_grp == j, st[SK * j:SK * (j + 1)], s)
            blocks.append(s)
        p_ref[64 * g:64 * (g + 1), :] = _softmax_t(blocks)


def _transpose_keys(k_ref, t, kt_ref):
    for b in range(B):
        ks = k_ref[b, HU * t:HU * (t + 1)].reshape(128, DH)
        kt_ref[b] = pltpu.bitcast(ks.T, U32)


def _scores_pv(q_refs, kt_ref, s_ref, p_ref, v_ref, t, o_ref, batches):
    lg = lax.broadcasted_iota(jnp.int32, (16, 128), 1) // 32
    lg32 = lax.broadcasted_iota(jnp.int32, (32, 128), 1) // 32
    zero = jnp.zeros((16, 128), U32)

    def keep(j, x):
        return jnp.where(lg != j, zero, x)

    def drop(j, x):
        return jnp.where(lg == j, zero, x)

    def mm(a, w):
        return jnp.dot(pltpu.bitcast(a, BF16), pltpu.bitcast(jnp.concatenate(w, axis=0), BF16),
                       preferred_element_type=F32)

    for b in batches:
        bs = (b + BP) % B
        kt = kt_ref[bs]
        vs = pltpu.bitcast(v_ref[b, HU * t:HU * (t + 1)].reshape(128, DH), U32)
        kc = [kt[16 * c:16 * (c + 1)] for c in range(4)]
        vc = [vs[16 * c:16 * (c + 1)] for c in range(4)]
        p = p_ref[16 * b:16 * (b + 1), :]
        qs = [pltpu.bitcast(q_refs[h][SQ * bs:SQ * (bs + 1), :], U32) for h in range(HU)]
        outs = []
        for j in range(4):
            w = [drop(j, vc[c]) if c == j else keep(j, kc[c]) for c in range(4)]
            outs.append(mm(jnp.where(lg == j, p, qs[j]), w))
        qd = qs[0]
        for j in range(1, 4):
            qd = jnp.where(lg == j, qs[j], qd)
        s_rest = mm(qd, [keep(c, kc[c]) for c in range(4)])
        o_rest = mm(p, [keep(c, vc[c]) for c in range(4)])
        s = outs[0]
        for j in range(1, 4):
            s = jnp.where(lg32 == j, outs[j], s)
        s_ref[SQ * bs:SQ * (bs + 1), :] = s + s_rest
        for j in range(4):
            o_ref[j, SQ * b:SQ * (b + 1), :] = jnp.where(lg32 == j, o_rest, outs[j]).astype(BF16)


def _store_heads(ref, h0, r):
    for h in range(r.shape[1] // DH):
        ref[h0 + h] = r[:, DH * h:DH * (h + 1)].astype(BF16)


def _kernel(xa, ka, va, wqa, woa, xb, kb, vb, wqb, wob, out_hbm,
            x_buf, wq_buf, wqn_buf, wo_buf, k0_buf, kv_buf,
            q_buf, qn_buf, p_buf, o_buf, kt_buf, s_buf, acc0, acc, out_buf, sems):
    xs, ks, vs, wqs, wos = (xa, xb), (ka, kb), (va, vb), (wqa, wqb), (woa, wob)

    def cp_piece(pc, s):
        if pc[0] == 'k':
            return pltpu.make_async_copy(ka.at[pl.ds(0, BP), pl.ds(0, HU)], k0_buf, sems.at[s])
        br = pc[1]
        k0, nk = pc[2] * DH, (pc[3] - pc[2]) * DH
        if pc[0] == 'x':
            return pltpu.make_async_copy(xs[br].at[:, pl.ds(k0, nk)], x_buf.at[br, :, pl.ds(k0, nk)], sems.at[s])
        v0, nh = pc[4], pc[5] - pc[4]
        h0 = v0 if v0 < HQ else v0 + HA
        return pltpu.make_async_copy(wqs[br].at[pl.ds(k0, nk), pl.ds(h0 * DH, nh * DH)],
                                     wq_buf.at[br, pl.ds(k0, nk), pl.ds(v0 * DH, nh * DH)], sems.at[s])

    def cp_wn(g):
        src = wqs[g // 2].at[:, pl.ds((g % 2) * GW + HQ * DH, HA * DH)]
        return pltpu.make_async_copy(src, wqn_buf.at[g], sems.at[S_WN + g])

    def cps_kv(g):
        sem = sems.at[S_KV + g]
        br, j = divmod(g, 2)
        lo, hi = pl.ds(0, BP), pl.ds(BP, B - BP)
        cps = [pltpu.make_async_copy(ks[br].at[hi, pl.ds(j * HG, HG)], kv_buf.at[g, 0, hi], sem)]
        if j == 0:
            cps += [pltpu.make_async_copy(ks[br].at[lo, pl.ds(HU, HG)], kv_buf.at[g, 0, lo], sem)]
        else:
            n = HG - HU
            cps += [pltpu.make_async_copy(ks[br].at[lo, pl.ds(HG + HU, n)], kv_buf.at[g, 0, lo, pl.ds(0, n)], sem),
                    pltpu.make_async_copy(ks[1 - br].at[lo, pl.ds(0, HU)], kv_buf.at[g, 0, lo, pl.ds(n, HU)], sem)]
        cps.append(pltpu.make_async_copy(vs[br].at[:, pl.ds(j * HG, HG)], kv_buf.at[g, 1], sem))
        return cps

    def wo_view(g):
        return wo_buf.at[g, :, pl.ds(0, D)]

    def cp_wo(g):
        return pltpu.make_async_copy(wos[g // 2].at[pl.ds((g % 2) * GW, GW), :], wo_view(g), sems.at[S_WO + g])

    def cp_out(br, i):
        c0, c1, r0, nr = _OUT_LIST[i]
        col = br * D + c0
        if not isinstance(col, int):
            col = pl.multiple_of(col, DH)
        return pltpu.make_async_copy(out_buf.at[br, pl.ds(r0, nr), pl.ds(c0, c1 - c0)],
                                     out_hbm.at[pl.ds(r0, nr), pl.ds(col, c1 - c0)],
                                     sems.at[S_OUT + br * len(_OUT_LIST) + i])

    def wait_fill(view, s):
        pltpu.make_async_copy(view, view, sems.at[s]).wait()

    def q_phase():
        s = 0
        for pcs in _PIECES:
            for pc in pcs:
                cp_piece(pc, s).start()
                s += 1
        for g in range(NG):
            cp_wn(g).start()
            for cp in cps_kv(g):
                cp.start()
            cp_wo(g).start()
        s = 0
        for reg, pcs in zip(REGIONS, _PIECES):
            for pc in pcs:
                cp_piece(pc, s).wait()
                s += 1
            for blk in reg:
                if blk == 'S':
                    _first_scores(q_buf, k0_buf, p_buf.at[0])
                    continue
                br, kt0, kt1, v0, v1 = blk
                k0, k1, n0, n1 = kt0 * DH, kt1 * DH, v0 * DH, v1 * DH
                r = jnp.dot(x_buf[br, :, k0:k1], wq_buf[br, k0:k1, n0:n1], preferred_element_type=F32)
                if k0 > 0:
                    r = acc0[:, n0:n1] + r
                if k1 < D:
                    acc0[:, n0:n1] = r
                else:
                    _store_heads(q_buf, br * 2 * HQ + v0, r)

    def a_step(g, carry):
        wait_fill(wqn_buf.at[g], S_WN + g)
        wait_fill(kv_buf.at[g], S_KV + g)
        wait_fill(wo_view(g), S_WO + g)
        br = g // 2
        last = (g % 2) == 1
        g_next = (g + 1) % NG

        def q_refs(u):
            if u < 3:
                return [q_buf.at[g * HQ + HU * u + h] for h in range(HU)]
            if u == 3:
                return [qn_buf.at[h] for h in range(HU)]
            return [q_buf.at[g_next * HQ + h] for h in range(HU)]

        def qproj(i):
            h0, h1 = i * HA // NP, (i + 1) * HA // NP
            r = jnp.dot(x_buf[br], wqn_buf[g, :, h0 * DH:h1 * DH], preferred_element_type=F32)
            _store_heads(qn_buf, h0, r)

        def keys(t):
            _transpose_keys(kv_buf.at[g, 0], t, kt_buf.at[t])

        def attn(t, i):
            u = t + 1 if i == NP - 1 else t
            _scores_pv(q_refs(u), kt_buf.at[t], s_buf.at[t], p_buf.at[t], kv_buf.at[g, 1], t, o_buf.at[t],
                       range(BP * i, BP * (i + 1)))
            nxt = (i + 1) % NP
            for r in range(nxt * BP // 4, (nxt + 1) * BP // 4):
                st = s_buf[t, 128 * r:128 * (r + 1), :].T
                p_buf[u % 4, 64 * r:64 * (r + 1), :] = _softmax_t(
                    [st[SK * h:SK * (h + 1)] for h in range(HU)])

        def o_lhs(t):
            return jnp.concatenate([o_buf[t, h] for h in range(HU)], axis=1)

        def oproj(t, i):
            n0, n1 = i * D // NP, (i + 1) * D // NP
            r = jnp.dot(o_lhs(t), wo_buf[g, UW * t:UW * (t + 1), n0:n1], preferred_element_type=F32)
            if t == 0:
                acc[:, n0:n1] = jnp.where(last, acc[:, n0:n1], 0.0) + r
            else:
                acc[:, n0:n1] += r

        def oproj_final():
            o = o_lhs(3)
            i = 0
            for (c0, c1, rs) in OUT_PIECES:
                r = jnp.dot(o, wo_buf[g, 3 * UW:4 * UW, c0:c1], preferred_element_type=F32)
                r = acc[:, c0:c1] + r
                acc[:, c0:c1] = r
                r = r.astype(BF16)
                r0 = 0
                for nr in rs:
                    out_buf[br, r0:r0 + nr, c0:c1] = r[r0:r0 + nr]
                    pl.when(last)(cp_out(br, i).start)
                    r0 += nr
                    i += 1

        keys(0)
        for i in range(NP):
            qproj(i)
            attn(0, i)
        for t in range(3):
            keys(t + 1)
            for i in range(NP):
                oproj(t, i)
                attn(t + 1, i)
        oproj_final()
        return carry

    def phase(s, carry):
        @pl.when(s == 0)
        def _():
            q_phase()
            lax.fori_loop(0, NG, a_step, 0)

        @pl.when(s == 1)
        def _():
            for br in range(2):
                for i in range(len(_OUT_LIST)):
                    cp_out(br, i).wait()
        return carry

    lax.fori_loop(0, 2, phase, 0)


@jax.jit
def pallas_concat_heads__mha_block_cached__mha_block_cached__near_ridge_kernel(
    A_x: jax.Array,
    A_k_cache: jax.Array,
    A_v_cache: jax.Array,
    A_wq: jax.Array,
    A_wo: jax.Array,
    B_x: jax.Array,
    B_k_cache: jax.Array,
    B_v_cache: jax.Array,
    B_wq: jax.Array,
    B_wo: jax.Array,
):
    any_spec = pl.BlockSpec(memory_space=pl.ANY)
    out = pl.pallas_call(
        _kernel,
        in_specs=[any_spec] * 10,
        out_specs=any_spec,
        out_shape=jax.ShapeDtypeStruct((M, 2 * D), BF16),
        scratch_shapes=[
            pltpu.VMEM((2, M, D), BF16),
            pltpu.VMEM((2, D, 2 * HQ * DH + PAD), BF16),
            pltpu.VMEM((NG, D, HA * DH), BF16),
            pltpu.VMEM((NG, GW, D + PAD), BF16),
            pltpu.VMEM((BP, HU, SK, DH), BF16),
            pltpu.VMEM((NG, 2, B, HG, SK, DH), BF16),
            pltpu.VMEM((NG * HQ, M, DH), BF16),
            pltpu.VMEM((HA, M, DH), BF16),
            pltpu.VMEM((4, M // 2, 128), U32),
            pltpu.VMEM((4, HU, M, DH), BF16),
            pltpu.VMEM((4, B, DH // 2, 128), U32),
            pltpu.VMEM((4, M, 128), F32),
            pltpu.VMEM((M, 2 * HQ * DH), F32),
            pltpu.VMEM((M, D), F32),
            pltpu.VMEM((2, M, D), BF16),
            pltpu.SemaphoreType.DMA((N_SEM,)),
        ],
        compiler_params=pltpu.CompilerParams(
            vmem_limit_bytes=100 * 1024 * 1024,
            disable_semaphore_checks=True,
            disable_bounds_checks=True,
        ),
    )(A_x.reshape(M, D), A_k_cache, A_v_cache, A_wq, A_wo,
      B_x.reshape(M, D), B_k_cache, B_v_cache, B_wq, B_wo)
    return out.reshape(B, SQ, 2 * D)
```
